```python
import os as _os
_os.environ.setdefault("JAX_PLATFORMS", "cpu")
import jax
import jax.numpy as jnp

def _softmax(x, axis=-1):
    return jax.nn.softmax(x, axis=axis)
def _gelu(x):
    return jax.nn.gelu(x, approximate=True)
def _silu(x):
    return jax.nn.silu(x)
def _sigmoid(x):
    return jax.nn.sigmoid(x)
def _layernorm(x, axis=-1, eps=1e-5):
    m = jnp.mean(x, axis=axis, keepdims=True)
    v = jnp.var(x, axis=axis, keepdims=True)
    return (x - m) / jnp.sqrt(v + eps)
def _scatter_add(tgt, idx, src, axis=0):
    return tgt.at[idx].add(src)
def _segment_sum(src, seg, n):
    return jax.ops.segment_sum(src, seg, n)
class _Rng:
    def __init__(self, key):
        self._k = key
    def _next(self):
        self._k, sub = jax.random.split(self._k)
        return sub
    def normal(self, shape):
        return jax.random.normal(self._next(), shape, dtype=jnp.bfloat16)
    def randint(self, lo, hi, shape):
        return jax.random.randint(self._next(), shape, lo, hi, dtype=jnp.int32)
    def uniform(self, shape, lo=0.0, hi=1.0):
        return jax.random.uniform(self._next(), shape, jnp.bfloat16, lo, hi)
    def permutation(self, n):
        return jax.random.permutation(self._next(), n)


kernel_name = 'parallel_sum__softmax_full_mha__swiglu_ffn__prompt'

def setup_inputs():
    _rng = _Rng(jax.random.key(int.from_bytes(__import__("os").urandom(4), "little")))
    _w = (lambda a: (lambda t: t.astype(jnp.bfloat16) if jnp.issubdtype(t.dtype, jnp.floating) else t)(jnp.asarray(a)))
    def _A_setup():
        B, S, D = 1, 2048, 640
        return {
            "x": _w((lambda *s: _rng.normal(s) * 0.05)(B, S, D)),
            "wqkv": _w((lambda *s: _rng.normal(s) * 0.1)(D, 3 * D)),
            "wo": _w((lambda *s: _rng.normal(s) * 0.05)(D, D)),
        }
    _A_in = _A_setup()

    def _B_setup():
        B, S, D, F = 1, 2048, 640, 1536
        return {
            "x": _w((lambda *s: _rng.normal(s) * 0.05)(B, S, D)),
            "w_gate": _w((lambda *s: _rng.normal(s) * 0.05)(D, F)),
            "w_up": _w((lambda *s: _rng.normal(s) * 0.05)(D, F)),
            "w_down": _w((lambda *s: _rng.normal(s) * 0.05)(F, D)),
        }
    _B_in = _B_setup()

    return {
        "A_x": _A_in["x"],
        "A_wqkv": _A_in["wqkv"],
        "A_wo": _A_in["wo"],
        "B_x": _B_in["x"],
        "B_w_gate": _B_in["w_gate"],
        "B_w_up": _B_in["w_up"],
        "B_w_down": _B_in["w_down"],
    }

def reference(A_x, A_wqkv, A_wo, B_x, B_w_gate, B_w_up, B_w_down):
    def _A_ref(x, wqkv, wo):
        B, S, D = x.shape
        H = 32; Dh = D // H
        qkv = (lambda x, *d: x.transpose(*d))((x @ wqkv).reshape(B, S, 3, H, Dh), 2, 0, 3, 1, 4)
        q, k, v = qkv[0], qkv[1], qkv[2]
        scale = Dh ** -0.5
        scores = jnp.einsum("bhqd,bhkd->bhqk", q, k) * scale
        p = _softmax(scores, axis=-1)
        o = jnp.einsum("bhqk,bhkd->bhqd", p, v)
        return (lambda x, *d: x.transpose(*d))(o, 0, 2, 1, 3).reshape(B, S, D) @ wo

    def _B_ref(x, w_gate, w_up, w_down):
        g = _silu(x @ w_gate)
        u = x @ w_up
        return (g * u) @ w_down

    x = A_x
    xn = _layernorm(x, axis=-1)
    return x + _A_ref(xn, A_wqkv, A_wo) + _B_ref(xn, B_w_gate, B_w_up, B_w_down)
```

```python
import functools, contextlib
import jax
import jax.numpy as jnp
from jax import lax
import jax.experimental.pallas as pl
import jax.experimental.pallas.tpu as pltpu

S, D, H, DH, F = 2048, 640, 32, 20, 1536
HPG = 6
NG = (H + HPG - 1) // HPG
VR = 24
LOG2E = 1.4426950408889634
NT = (((1,), (1,)), ((), ()))
TN = (((0,), (0,)), ((), ()))
TT = (((0,), (1,)), ((), ()))
f32, bf16 = jnp.float32, jnp.bfloat16


def body(x_h, wqkv_h, wo_h, wg_h, wu_h, wd_h, o_h,
         x_s, wqkv_s, wo_s, wg_s, wu_s, wd_s, out_s,
         xn_s, qt_s, k_s, vt_s, s_s, m_s, ot_s, sems, osems, *, QT, CH, U, RB, FC, PB, SC):
    ns = jax.named_scope if SC else (lambda n: contextlib.nullcontext())
    NPB = S // PB
    xcp = [pltpu.make_async_copy(x_h.at[pl.ds(i * PB, PB)], x_s.at[pl.ds(i * PB, PB)], sems.at[5 + i]) for i in range(NPB)]
    wcp = [pltpu.make_async_copy(a, b, sems.at[i]) for i, (a, b) in enumerate(
        ((wqkv_h, wqkv_s), (wo_h, wo_s), (wg_h, wg_s), (wu_h, wu_s), (wd_h, wd_s)))]
    xcp[0].start()
    wcp[0].start()
    for c in xcp[1:]:
        c.start()
    for c in wcp[1:]:
        c.start()

    with ns('prol'):
        qt_s[D:, :] = jnp.zeros((qt_s.shape[0] - D, S), f32)
        tail = (lax.broadcasted_iota(jnp.int32, (VR - DH, PB), 0) == 0).astype(f32)
        for b in range(NPB):
            rows = slice(b * PB, (b + 1) * PB)
            xcp[b].wait()
            x = x_s[rows, :].astype(f32)
            mu = jnp.mean(x, axis=-1, keepdims=True)
            xc = x - mu
            var = jnp.mean(xc * xc, axis=-1, keepdims=True)
            xn = (xc * lax.rsqrt(var + 1e-5)).astype(bf16)
            xn_s[rows, :] = xn
            if b == 0:
                wcp[0].wait()
            k = jnp.dot(xn, wqkv_s[:, D:2 * D], preferred_element_type=f32)
            for g in range(NG):
                lo = g * HPG * DH
                w = min(128, D - lo)
                kg = k[:, lo:lo + w]
                if w < 128:
                    kg = jnp.concatenate([kg, jnp.zeros((PB, 128 - w), f32)], axis=1)
                k_s[g, rows, :] = kg.astype(bf16)
            qt = lax.dot_general(wqkv_s[:, 0:D], xn, TT, preferred_element_type=f32)
            qt_s[0:D, rows] = qt * (DH ** -0.5 * LOG2E)
            vt = lax.dot_general(wqkv_s[:, 2 * D:3 * D], xn, TT, preferred_element_type=f32)
            for h in range(H):
                vt_s[h, :, rows] = jnp.concatenate([vt[h * DH:(h + 1) * DH], tail], axis=0)

    NQ = S // QT
    NC = S // CH

    def cols(t):
        return pl.ds(pl.multiple_of((t // H) * QT, QT), QT)

    def stage(tq, tp, slot):
        if tq is not None:
            hq = tq % H
            g = hq // HPG
            j = hq - g * HPG
            qw = qt_s[pl.ds(pl.multiple_of(g * (HPG * DH), 8), 128), cols(tq)]
            r = lax.broadcasted_iota(jnp.int32, (128, QT), 0) - j * DH
            qw = jnp.where((r >= 0) & (r < DH), qw, 0.0).astype(bf16)
        if tp is not None:
            hp = tp % H
            m = m_s[slot]
        mx = o = None
        for c in range(NC):
            rows = slice(c * CH, (c + 1) * CH)
            if tq is not None:
                s = jnp.dot(k_s[g, rows, :], qw, preferred_element_type=f32)
                s_s[1 - slot, rows, :] = s
                cm = jnp.max(s.reshape(CH // 8, 8, QT), axis=0)
                mx = cm if mx is None else jnp.maximum(mx, cm)
            if tp is not None:
                p = jnp.exp2(s_s[slot, rows, :] - m)
                oc = jnp.dot(vt_s[hp, :, rows], p, preferred_element_type=f32)
                o = oc if o is None else o + oc
        if tq is not None:
            m_s[1 - slot] = jnp.max(mx, axis=0, keepdims=True)
        if tp is not None:
            ot_s[hp, :, cols(tp)] = o * (1.0 / o[DH:DH + 1])

    T = NQ * H
    with ns('att'):
        stage(0, None, 1)
        n_loop = (T - 1) // U
        def step(i, c):
            for u in range(U):
                stage(i * U + u + 1, i * U + u, u % 2)
            return c
        lax.fori_loop(0, n_loop, step, 0)
        for t in range(n_loop * U, T - 1):
            stage(t + 1, t, t % 2)
        stage(None, T - 1, (T - 1) % 2)

    for c in wcp[1:]:
        c.wait()

    def ocp(i):
        return pltpu.make_async_copy(out_s.at[i], o_h.at[pl.ds(i * RB, RB)], osems.at[i])

    with ns('ffn'):
        def fstep(i, c):
            r0 = pl.multiple_of(i * RB, RB)
            rows = pl.ds(r0, RB)
            ot = jnp.concatenate([ot_s[h, 0:DH, rows] for h in range(H)], axis=0).astype(bf16)
            acc = x_s[rows, :].astype(f32) + lax.dot_general(ot, wo_s[...], TN, preferred_element_type=f32)
            xn = xn_s[rows, :]
            for f in range(F // FC):
                fc = slice(f * FC, (f + 1) * FC)
                gate = jnp.dot(xn, wg_s[:, fc], preferred_element_type=f32)
                up = jnp.dot(xn, wu_s[:, fc], preferred_element_type=f32)
                act = (gate * jax.nn.sigmoid(gate) * up).astype(bf16)
                acc = acc + jnp.dot(act, wd_s[fc, :], preferred_element_type=f32)
            out_s[i] = acc.astype(out_s.dtype)
            ocp(i).start()
            return c
        lax.fori_loop(0, S // RB, fstep, 0)
        for i in range(S // RB):
            ocp(i).wait()


def make(QT=512, CH=128, U=4, RB=256, FC=512, PB=512, SC=False):
    @jax.jit
    def run(A_x, A_wqkv, A_wo, B_x, B_w_gate, B_w_up, B_w_down):
        x = A_x.reshape(S, D)
        ins = (x, A_wqkv, A_wo, B_w_gate, B_w_up, B_w_down)
        out = pl.pallas_call(
            functools.partial(body, QT=QT, CH=CH, U=U, RB=RB, FC=FC, PB=PB, SC=SC),
            in_specs=[pl.BlockSpec(memory_space=pl.ANY) for a in ins],
            out_specs=pl.BlockSpec(memory_space=pl.ANY),
            out_shape=jax.ShapeDtypeStruct((S, D), A_x.dtype),
            scratch_shapes=[pltpu.VMEM(a.shape, a.dtype) for a in ins] + [
                pltpu.VMEM((S // RB, RB, D), A_x.dtype),
                pltpu.VMEM((S, D), bf16),
                pltpu.VMEM(((NG - 1) * HPG * DH + 128, S), f32),
                pltpu.VMEM((NG, S, 128), bf16),
                pltpu.VMEM((H, VR, S), f32),
                pltpu.VMEM((2, S, QT), f32),
                pltpu.VMEM((2, 1, QT), f32),
                pltpu.VMEM((H, VR, S), f32),
                pltpu.SemaphoreType.DMA((5 + S // PB,)),
                pltpu.SemaphoreType.DMA((S // RB,)),
            ],
            compiler_params=pltpu.CompilerParams(vmem_limit_bytes=110 * 2**20),
        )(*ins)
        return out.reshape(1, S, D)
    return run


_run = make()


def pallas_parallel_sum__softmax_full_mha__swiglu_ffn__prompt_kernel(
    A_x, A_wqkv, A_wo, B_x, B_w_gate, B_w_up, B_w_down
):
    return _run(A_x, A_wqkv, A_wo, B_x, B_w_gate, B_w_up, B_w_down)
```

```python
import functools, contextlib
import jax
import jax.numpy as jnp
from jax import lax
import jax.experimental.pallas as pl
import jax.experimental.pallas.tpu as pltpu

S, D, H, DH, F = 2048, 640, 32, 20, 1536
VR = 24
LOG2E = 1.4426950408889634
NT = (((1,), (1,)), ((), ()))
TN = (((0,), (0,)), ((), ()))
TT = (((0,), (1,)), ((), ()))
f32, bf16 = jnp.float32, jnp.bfloat16


def body(x_h, wqkv_h, wo_h, wg_h, wu_h, wd_h, o_h,
         x_s, wqkv_s, wo_s, wg_s, wu_s, wd_s, out_s,
         xn_s, qt_s, k_s, vt_s, s_s, m_s, ot_s, sems, osems, *, QT, CH, U, RB, FC, PB, SC, PF):
    ns = jax.named_scope if SC else (lambda n: contextlib.nullcontext())
    NPB = S // PB
    xcp = [pltpu.make_async_copy(x_h.at[pl.ds(i * PB, PB)], x_s.at[pl.ds(i * PB, PB)], sems.at[7 + i]) for i in range(NPB)]
    wcp = [pltpu.make_async_copy(a, b, sems.at[i]) for i, (a, b) in enumerate(
        ((wo_h, wo_s), (wg_h, wg_s), (wu_h, wu_s), (wd_h, wd_s)))]
    pcp = [pltpu.make_async_copy(wqkv_h.at[:, pl.ds(i * D, D)], wqkv_s.at[:, pl.ds(i * D, D)], sems.at[4 + i]) for i in range(3)]
    xcp[0].start()
    pcp[1].start()
    pcp[0].start()
    pcp[2].start()
    for c in xcp[1:]:
        c.start()

    with ns('prol'):
        tail = (lax.broadcasted_iota(jnp.int32, (VR - DH, PB), 0) == 0).astype(f32)
        def ln(b):
            rows = slice(b * PB, (b + 1) * PB)
            xcp[b].wait()
            x = x_s[rows, :].astype(f32)
            mu = jnp.mean(x, axis=-1, keepdims=True)
            xc = x - mu
            var = jnp.mean(xc * xc, axis=-1, keepdims=True)
            xn_s[rows, :] = (xc * lax.rsqrt(var + 1e-5)).astype(bf16)

        ln(0)
        for b in range(NPB):
            rows = slice(b * PB, (b + 1) * PB)
            xn = xn_s[rows, :]
            if b == 0:
                pcp[1].wait()
            k = jnp.dot(xn, wqkv_s[:, D:2 * D], preferred_element_type=f32)
            k = jnp.concatenate([k, jnp.zeros((PB, 128), f32)], axis=1)
            if b == 0:
                pcp[0].wait()
                pcp[2].wait()
                for c in wcp:
                    c.start()
            if b + 1 < NPB:
                ln(b + 1)
            G = 640
            for j in range(1):
                qt = lax.dot_general(wqkv_s[:, j * G:(j + 1) * G], xn, TT, preferred_element_type=f32) * (DH ** -0.5 * LOG2E)
                vt = lax.dot_general(wqkv_s[:, 2 * D + j * G:2 * D + (j + 1) * G], xn, TT, preferred_element_type=f32)
                for i in range(G // DH):
                    h = j * (G // DH) + i
                    k_s[h, rows, :] = k[:, h * DH:h * DH + 32].astype(bf16)
                    qt_s[h, :, rows] = jnp.concatenate([qt[i * DH:(i + 1) * DH], jnp.zeros((32 - DH, PB), f32)], axis=0).astype(bf16)
                    vt_s[h, :, rows] = jnp.concatenate([vt[i * DH:(i + 1) * DH], tail], axis=0)

    NQ = S // QT
    NC = S // CH

    def cols(t):
        return pl.ds(pl.multiple_of((t // H) * QT, QT), QT)

    def stage(tq, tp, slot):
        if tq is not None:
            hq = tq % H
            qw = qt_s[hq, :, cols(tq)]
        if tp is not None:
            hp = tp % H
            m = m_s[slot]
        mx = o = None
        for c in range(NC):
            rows = slice(c * CH, (c + 1) * CH)
            if tp is not None and PF:
                p = jnp.exp2(s_s[slot, rows, :] - m)
                oc = lax.dot_general(vt_s[hp, :, rows], p.astype(bf16), (((1,), (0,)), ((), ())), preferred_element_type=f32)
                o = oc if o is None else o + oc
            if tq is not None:
                s = jnp.dot(k_s[hq, rows, :], qw, preferred_element_type=f32)
                s_s[1 - slot, rows, :] = s
                cm = jnp.max(s.reshape(CH // 8, 8, QT), axis=0)
                mx = cm if mx is None else jnp.maximum(mx, cm)
            if tp is not None and not PF:
                p = jnp.exp2(s_s[slot, rows, :] - m)
                oc = lax.dot_general(vt_s[hp, :, rows], p.astype(bf16), (((1,), (0,)), ((), ())), preferred_element_type=f32)
                o = oc if o is None else o + oc
        if tq is not None:
            m_s[1 - slot] = jnp.max(mx, axis=0, keepdims=True)
        if tp is not None:
            ot_s[hp, :, cols(tp)] = o * (1.0 / o[DH:DH + 1])

    T = NQ * H
    with ns('att'):
        stage(0, None, 1)
        n_loop = (T - 1) // U
        def step(i, c):
            for u in range(U):
                stage(i * U + u + 1, i * U + u, u % 2)
            return c
        lax.fori_loop(0, n_loop, step, 0)
        for t in range(n_loop * U, T - 1):
            stage(t + 1, t, t % 2)
        stage(None, T - 1, (T - 1) % 2)

    for c in wcp:
        c.wait()

    def ocp(i):
        return pltpu.make_async_copy(out_s.at[i], o_h.at[pl.ds(i * RB, RB)], osems.at[i])

    with ns('ffn'):
        def fstep(i, c):
            r0 = pl.multiple_of(i * RB, RB)
            rows = pl.ds(r0, RB)
            ot = jnp.concatenate([ot_s[h, 0:DH, rows] for h in range(H)], axis=0).astype(bf16)
            acc = x_s[rows, :].astype(f32) + lax.dot_general(ot, wo_s[...], TN, preferred_element_type=f32)
            xn = xn_s[rows, :]
            for f in range(F // FC):
                fc = slice(f * FC, (f + 1) * FC)
                gate = jnp.dot(xn, wg_s[:, fc], preferred_element_type=f32)
                up = jnp.dot(xn, wu_s[:, fc], preferred_element_type=f32)
                act = (gate * jax.nn.sigmoid(gate) * up).astype(bf16)
                acc = acc + jnp.dot(act, wd_s[fc, :], preferred_element_type=f32)
            out_s[i] = acc.astype(out_s.dtype)
            ocp(i).start()
            return c
        lax.fori_loop(0, S // RB, fstep, 0)
        for i in range(S // RB):
            ocp(i).wait()


def make(QT=512, CH=128, U=8, RB=512, FC=512, PB=1024, SC=False, PF=False, FL={}):
    @jax.jit
    def run(A_x, A_wqkv, A_wo, B_x, B_w_gate, B_w_up, B_w_down):
        x = A_x.reshape(S, D)
        ins = (x, A_wqkv, A_wo, B_w_gate, B_w_up, B_w_down)
        out = pl.pallas_call(
            functools.partial(body, QT=QT, CH=CH, U=U, RB=RB, FC=FC, PB=PB, SC=SC, PF=PF),
            in_specs=[pl.BlockSpec(memory_space=pl.ANY) for a in ins],
            out_specs=pl.BlockSpec(memory_space=pl.ANY),
            out_shape=jax.ShapeDtypeStruct((S, D), A_x.dtype),
            scratch_shapes=[pltpu.VMEM(a.shape, a.dtype) for a in ins] + [
                pltpu.VMEM((S // RB, RB, D), A_x.dtype),
                pltpu.VMEM((S, D), bf16),
                pltpu.VMEM((H, 32, S), bf16),
                pltpu.VMEM((H, S, 32), bf16),
                pltpu.VMEM((H, VR, S), f32),
                pltpu.VMEM((2, S, QT), f32),
                pltpu.VMEM((2, 1, QT), f32),
                pltpu.VMEM((H, VR, S), f32),
                pltpu.SemaphoreType.DMA((7 + S // PB,)),
                pltpu.SemaphoreType.DMA((S // RB,)),
            ],
            compiler_params=pltpu.CompilerParams(vmem_limit_bytes=110 * 2**20, flags=FL),
        )(*ins)
        return out.reshape(1, S, D)
    return run


_run = make()


def pallas_parallel_sum__softmax_full_mha__swiglu_ffn__prompt_kernel(
    A_x, A_wqkv, A_wo, B_x, B_w_gate, B_w_up, B_w_down
):
    return _run(A_x, A_wqkv, A_wo, B_x, B_w_gate, B_w_up, B_w_down)
```
